```python
import jax
import jax.numpy as jnp

def _softmax(x, axis=-1):
    return jax.nn.softmax(x, axis=axis)
def _gelu(x):
    return jax.nn.gelu(x, approximate=True)
def _silu(x):
    return jax.nn.silu(x)
def _sigmoid(x):
    return jax.nn.sigmoid(x)
def _layernorm(x, axis=-1, eps=1e-5):
    m = jnp.mean(x, axis=axis, keepdims=True)
    v = jnp.var(x, axis=axis, keepdims=True)
    return (x - m) / jnp.sqrt(v + eps)
def _scatter_add(tgt, idx, src, axis=0):
    return tgt.at[idx].add(src)
def _segment_sum(src, seg, n):
    return jax.ops.segment_sum(src, seg, n)
class _Rng:
    def __init__(self, key):
        self._k = key
    def _next(self):
        self._k, sub = jax.random.split(self._k)
        return sub
    def normal(self, shape):
        return jax.random.normal(self._next(), shape, dtype=jnp.bfloat16)
    def randint(self, lo, hi, shape):
        return jax.random.randint(self._next(), shape, lo, hi, dtype=jnp.int32)
    def uniform(self, shape, lo=0.0, hi=1.0):
        return jax.random.uniform(self._next(), shape, jnp.bfloat16, lo, hi)
    def permutation(self, n):
        return jax.random.permutation(self._next(), n)


kernel_name = 'interleave_layers__sliding_block_cached__dense_activation_gelu__decode'

def _fwd_setup_inputs():
    _rng = _Rng(jax.random.key(int.from_bytes(__import__("os").urandom(4), "little")))
    _w = (lambda a: (lambda t: t.astype(jnp.bfloat16) if jnp.issubdtype(t.dtype, jnp.floating) else t)(jnp.asarray(a)))
    def _A_setup():
        B, Sq, D = 2, 1, 512
        Hq, Hkv, Sk, Dh = 32, 8, 32768, 128
        assert Hq % Hkv == 0, (Hq, Hkv)
        return {
            "x": _w((lambda *s: _rng.normal(s) * 0.05)(B, Sq, D)),
            "k_cache": _w((lambda *s: _rng.normal(s) * 0.05)(B, Hkv, Sk, Dh)),
            "v_cache": _w((lambda *s: _rng.normal(s) * 0.05)(B, Hkv, Sk, Dh)),
            "wq": _w((lambda *s: _rng.normal(s) * 0.05)(D, Hq * Dh) * (D ** -0.5)),
            "wo": _w((lambda *s: _rng.normal(s) * 0.05)(Hq * Dh, D) * ((Hq * Dh) ** -0.5)),
        }
    _A_in = _A_setup()

    def _B_setup():
        B, S, D, F = 2, 1, 512, 1792
        return {
            "x": _w((lambda *s: _rng.normal(s) * 0.05)(B, S, D)),
            "w1": _w((lambda *s: _rng.normal(s) * 0.05)(D, F) * (D ** -0.5)),
            "b1": _w((lambda *s: _rng.normal(s) * 0.05)(F) * 0.01),
            "w2": _w((lambda *s: _rng.normal(s) * 0.05)(F, D) * (F ** -0.5)),
            "b2": _w((lambda *s: _rng.normal(s) * 0.05)(D) * 0.01),
        }
    _B_in = _B_setup()

    return {
        "A_x": _A_in["x"],
        "A_k_cache": _A_in["k_cache"],
        "A_v_cache": _A_in["v_cache"],
        "A_wq": _A_in["wq"],
        "A_wo": _A_in["wo"],
        "B_x": _B_in["x"],
        "B_w1": _B_in["w1"],
        "B_b1": _B_in["b1"],
        "B_w2": _B_in["w2"],
        "B_b2": _B_in["b2"],
    }

def _fwd_reference(A_x, A_k_cache, A_v_cache, A_wq, A_wo, B_x, B_w1, B_b1, B_w2, B_b2):
    def _A_ref(x, k_cache, v_cache, wq, wo):
        B, Sq, D = x.shape
        Hq, Dh = 32, 128
        Hkv, Sk = k_cache.shape[1], k_cache.shape[2]
        W = min(4096, max(256, Sk // 4))
        rep = Hq // Hkv
        q = (lambda x, *d: x.transpose(*d))((x @ wq).reshape(B, Sq, Hq, Dh), 0, 2, 1, 3)
        k = jnp.repeat(k_cache[:, :, Sk - W:, :], rep, axis=1)
        v = jnp.repeat(v_cache[:, :, Sk - W:, :], rep, axis=1)
        scores = jnp.einsum("bhqd,bhkd->bhqk", q, k) * (Dh ** -0.5)
        p = _softmax(scores, axis=-1)
        o = jnp.einsum("bhqk,bhkd->bhqd", p, v)
        return (lambda x, *d: x.transpose(*d))(o, 0, 2, 1, 3).reshape(B, Sq, Hq * Dh) @ wo

    def _B_ref(x, w1, b1, w2, b2):
        h = jnp.einsum("bsd,df->bsf", x, w1) + b1
        h = _gelu(h)
        return jnp.einsum("bsf,fd->bsd", h, w2) + b2

    x = A_x
    x = x + _A_ref(_layernorm(x, axis=-1), A_k_cache, A_v_cache, A_wq, A_wo)
    x = x + _B_ref(_layernorm(x, axis=-1), B_w1, B_b1, B_w2, B_b2)
    x = x + _A_ref(_layernorm(x, axis=-1), A_k_cache, A_v_cache, A_wq, A_wo)
    x = x + _B_ref(_layernorm(x, axis=-1), B_w1, B_b1, B_w2, B_b2)
    return x


def setup_inputs():
    _inp = _fwd_setup_inputs()
    _gk = jax.random.fold_in(jax.random.key(int.from_bytes(__import__("os").urandom(4), "little")), 2**31 - 1)
    _shapes = [[2, 1, 512]]
    _dtypes = ['bfloat16']
    _gks = jax.random.split(_gk, len(_shapes))
    _gs = [jax.random.normal(k, s, dtype=jnp.dtype(d)) * 0.05 for k, s, d in zip(_gks, _shapes, _dtypes)]
    _inp["grad_out"] = _gs[0]
    return _inp

def reference(A_x, A_k_cache, A_v_cache, A_wq, A_wo, B_w1, B_b1, B_w2, B_b2, B_x, grad_out):
    _const = dict(B_x=B_x)
    def _f(*_d):
        return _fwd_reference(**{'A_x': _d[0], 'A_k_cache': _d[1], 'A_v_cache': _d[2], 'A_wq': _d[3], 'A_wo': _d[4], 'B_w1': _d[5], 'B_b1': _d[6], 'B_w2': _d[7], 'B_b2': _d[8], **_const})
    _out, _vjp = jax.vjp(_f, A_x, A_k_cache, A_v_cache, A_wq, A_wo, B_w1, B_b1, B_w2, B_b2)
    _grads = _vjp(grad_out)
    _out0 = jnp.asarray(_out)
    return (_out0, *[jnp.asarray(_g) for _g in _grads])
```

```python
import math

import jax
import jax.numpy as jnp
import jax.experimental.pallas as pl
import jax.experimental.pallas.tpu as pltpu

_F32 = jnp.float32
_BF16 = jnp.bfloat16

_ZROWS = 128
_ZHEADS = 4


def _mm(a, b):
    return jax.lax.dot_general(a, b, (((1,), (0,)), ((), ())), preferred_element_type=_F32)


def _mm_nt(a, b):
    return jax.lax.dot_general(a, b, (((1,), (1,)), ((), ())), preferred_element_type=_F32)


def _ln_fwd(x, eps=1e-5):
    xc = x - jnp.mean(x, axis=-1, keepdims=True)
    var = jnp.mean(xc * xc, axis=-1, keepdims=True)
    rstd = 1.0 / jnp.sqrt(var + eps)
    return xc * rstd, rstd


def _ln_bwd(dy, y, rstd):
    return rstd * (dy - jnp.mean(dy, axis=-1, keepdims=True)
                   - y * jnp.mean(dy * y, axis=-1, keepdims=True))


_GELU_C = math.sqrt(2.0 / math.pi)
_GELU_A = 0.044715


def _gelu_and_grad(h):
    t = jnp.tanh(_GELU_C * (h + _GELU_A * h * h * h))
    cdf = 0.5 * (1.0 + t)
    dcdf = 0.5 * (1.0 - t * t) * _GELU_C * (1.0 + 3.0 * _GELU_A * h * h)
    return h * cdf, cdf + h * dcdf


@jax.jit
def pallas_interleave_layers__sliding_block_cached__dense_activation_gelu__decode_kernel(
    A_x: jax.Array,
    A_k_cache: jax.Array,
    A_v_cache: jax.Array,
    A_wq: jax.Array,
    A_wo: jax.Array,
    B_x: jax.Array,
    B_w1: jax.Array,
    B_b1: jax.Array,
    B_w2: jax.Array,
    B_b2: jax.Array,
    grad_out: jax.Array,
):
    del B_x
    B, Sq, D = A_x.shape
    _, Hkv, Sk, Dh = A_k_cache.shape
    HD = A_wq.shape[1]
    Hq = HD // Dh
    F = B_w1.shape[1]
    W = min(4096, max(256, Sk // 4))
    REP = Hq // Hkv
    R = B * REP
    NL = 2
    G = NL * Hkv * R
    assert (B, Sq, REP, R, Dh, G) == (2, 1, 4, 8, 128, 128)
    assert Hkv % _ZHEADS == 0 and (Sk - W) % _ZROWS == 0 and W % _ZROWS == 0
    scale = Dh ** -0.5
    NG = B * Hkv // _ZHEADS
    NZJ = (Sk - W) // _ZROWS
    NWJ = W // _ZROWS
    NZ = NG * NZJ

    def kernel(x_hbm, k_hbm, v_hbm, wq_hbm, wo_hbm, w1_hbm, b1_hbm, w2_hbm, b2_hbm, g_hbm,
               out_hbm, dx_hbm, dk_hbm, dv_hbm, dwq_hbm, dwo_hbm, dw1_hbm, db1_hbm, dw2_hbm, db2_hbm,
               k_v, v_v, wq_v, wo_v, w1_v, w2_v, x_v, g_v, b1_v, b2_v,
               dk_v, dv_v, dwq_v, dwo_v, dw1_v, dw2_v, out_v, dx_v, db1_v, db2_v,
               zero_v, p_s, ds_s, pt_s, dst_s, q_s, o_s, do_s, dq_s,
               rsem, wsem):
        reads = [
            pltpu.make_async_copy(k_hbm.at[:, :, pl.ds(Sk - W, W), :], k_v, rsem.at[0]),
            pltpu.make_async_copy(v_hbm.at[:, :, pl.ds(Sk - W, W), :], v_v, rsem.at[1]),
            pltpu.make_async_copy(x_hbm, x_v, rsem.at[2]),
            pltpu.make_async_copy(g_hbm, g_v, rsem.at[3]),
            pltpu.make_async_copy(b1_hbm, b1_v, rsem.at[4]),
            pltpu.make_async_copy(b2_hbm, b2_v, rsem.at[5]),
            pltpu.make_async_copy(wq_hbm, wq_v, rsem.at[6]),
            pltpu.make_async_copy(wo_hbm, wo_v, rsem.at[7]),
            pltpu.make_async_copy(w1_hbm, w1_v, rsem.at[8]),
            pltpu.make_async_copy(w2_hbm, w2_v, rsem.at[9]),
        ]
        for c in reads:
            c.start()
        zero_v[...] = jnp.zeros(zero_v.shape, zero_v.dtype)
        for c in reads:
            c.wait()

        def cache_write(src, dst_hbm, grp, row0):
            b, h0 = grp // (Hkv // _ZHEADS), (grp % (Hkv // _ZHEADS)) * _ZHEADS
            return pltpu.make_async_copy(
                src, dst_hbm.at[b, pl.ds(h0, _ZHEADS), pl.ds(row0, _ZROWS), :], wsem)

        def zero_write(dst_hbm, z):
            return cache_write(zero_v, dst_hbm, z // NZJ,
                               pl.multiple_of((z % NZJ) * _ZROWS, _ZROWS))

        issued = [0]

        def pump(n, i=0, trips=1):
            base = issued[0]
            assert base + n * trips <= NZ
            for j in range(n):
                zero_write(dk_hbm, base + i * n + j).start()
            issued[0] = base + n * trips

        row = jax.lax.broadcasted_iota(jnp.int32, (R, 1), 0)
        first_b = row < REP
        row_r = row % REP

        def per_batch(a0, a1):
            return jnp.where(first_b, a0, a1)

        def load_rep(ref):
            return per_batch(ref[0].astype(_F32), ref[1].astype(_F32))

        def sum_r(a):
            s0 = jnp.sum(jnp.where(first_b, a, 0.0), axis=0, keepdims=True)
            s1 = jnp.sum(jnp.where(first_b, 0.0, a), axis=0, keepdims=True)
            return per_batch(s0, s1)

        def store_heads(dst, l, a_rep):
            for h in range(Hkv):
                t = a_rep[:, (h * REP) * Dh:(h * REP + 1) * Dh]
                for r in range(1, REP):
                    t = jnp.where(row_r == r, a_rep[:, (h * REP + r) * Dh:(h * REP + r + 1) * Dh], t)
                dst[pl.ds((l * Hkv + h) * R, R), :] = t

        def load_masked(src, l):
            parts = []
            for h in range(Hkv):
                t = src[pl.ds((l * Hkv + h) * R, R), :]
                parts += [jnp.where(row_r == r, t, 0.0) for r in range(REP)]
            return jnp.concatenate(parts, axis=1).astype(_BF16)

        def attn_fwd(l):
            def body(h, carry):
                pump(ATT_PUMP, h, Hkv)
                rows = pl.ds(pl.multiple_of((l * Hkv + h) * R, R), R)
                q = q_s[rows, :].astype(_BF16)
                s = per_batch(_mm_nt(q, k_v[0, h]), _mm_nt(q, k_v[1, h])) * scale
                e = jnp.exp(s - jnp.max(s, axis=-1, keepdims=True))
                p = e / jnp.sum(e, axis=-1, keepdims=True)
                p_s[rows, :] = p
                pb = p.astype(_BF16)
                o_s[rows, :] = per_batch(_mm(pb, v_v[0, h]), _mm(pb, v_v[1, h]))
                return carry
            jax.lax.fori_loop(0, Hkv, body, 0)

        def attn_bwd(l):
            def body(h, carry):
                pump(ATT_PUMP, h, Hkv)
                rows = pl.ds(pl.multiple_of((l * Hkv + h) * R, R), R)
                do = do_s[rows, :].astype(_BF16)
                dp = per_batch(_mm_nt(do, v_v[0, h]), _mm_nt(do, v_v[1, h]))
                p = p_s[rows, :]
                ds = p * (dp - jnp.sum(p * dp, axis=-1, keepdims=True)) * scale
                ds_s[rows, :] = ds
                dsb = ds.astype(_BF16)
                dq_s[rows, :] = per_batch(_mm(dsb, k_v[0, h]), _mm(dsb, k_v[1, h]))
                return carry
            jax.lax.fori_loop(0, Hkv, body, 0)

        ATT_PUMP = 12
        pump(32)
        b1 = b1_v[...].astype(_F32).reshape(1, F)
        b2 = b2_v[...].astype(_F32).reshape(1, D)

        x = load_rep(x_v)
        saved = []
        for l in range(NL):
            ya, rstd_a = _ln_fwd(x)
            ya_b = ya.astype(_BF16)
            store_heads(q_s, l, _mm(ya_b, wq_v[...]))
            pump(8)
            attn_fwd(l)
            o_b = load_masked(o_s, l)
            x = x + sum_r(_mm(o_b, wo_v[...]))
            pump(8)
            yb, rstd_b = _ln_fwd(x)
            yb_b = yb.astype(_BF16)
            act, dact = _gelu_and_grad(_mm(yb_b, w1_v[...]) + b1)
            act_b = act.astype(_BF16)
            x = x + _mm(act_b, w2_v[...]) + b2
            pump(8)
            saved.append((ya, rstd_a, ya_b, o_b, yb, rstd_b, yb_b, act_b, dact))
        out_v[0] = x[0:1].astype(_BF16)
        out_v[1] = x[REP:REP + 1].astype(_BF16)

        once = row_r == 0
        dx = load_rep(g_v)
        db1 = jnp.zeros((1, F), _F32)
        db2 = jnp.zeros((1, D), _F32)
        wq_ops, wo_ops, w1_ops, w2_ops = [], [], [], []
        for l in reversed(range(NL)):
            ya, rstd_a, ya_b, o_b, yb, rstd_b, yb_b, act_b, dact = saved[l]
            dx_once = jnp.where(once, dx, 0.0)
            db2 = db2 + jnp.sum(dx_once, axis=0, keepdims=True)
            w2_ops.append((act_b, dx_once.astype(_BF16)))
            dh = _mm_nt(dx.astype(_BF16), w2_v[...]) * dact
            dh_once = jnp.where(once, dh, 0.0)
            db1 = db1 + jnp.sum(dh_once, axis=0, keepdims=True)
            w1_ops.append((yb_b, dh_once.astype(_BF16)))
            dx = dx + _ln_bwd(_mm_nt(dh.astype(_BF16), w1_v[...]), yb, rstd_b)
            pump(8)
            dx_b = dx.astype(_BF16)
            wo_ops.append((o_b, dx_b))
            store_heads(do_s, l, _mm_nt(dx_b, wo_v[...]))
            pump(8)
            attn_bwd(l)
            dq_b = load_masked(dq_s, l)
            wq_ops.append((ya_b, dq_b))
            dx = dx + _ln_bwd(sum_r(_mm_nt(dq_b, wq_v[...])), ya, rstd_a)
            pump(8)
        dx_v[0] = dx[0:1].astype(_BF16)
        dx_v[1] = dx[REP:REP + 1].astype(_BF16)
        db1_v[...] = db1.reshape(F).astype(_BF16)
        db2_v[...] = db2.reshape(D).astype(_BF16)

        def weight_grad(dst, ops):
            a = jnp.concatenate([o[0].astype(_F32) for o in ops], axis=0)
            b = jnp.concatenate([o[1] for o in ops], axis=0)
            n, m = dst.shape
            for i in range(0, n, 512):
                sz = min(512, n - i)
                at = a[:, i:i + sz].T.astype(_BF16)
                for j in range(0, m, 1024):
                    sm = min(1024, m - j)
                    dst[i:i + sz, j:j + sm] = _mm(at, b[:, j:j + sm]).astype(_BF16)
                    pump(2)

        weight_grad(dwq_v, wq_ops)
        weight_grad(dwo_v, wo_ops)
        weight_grad(dw1_v, w1_ops)
        weight_grad(dw2_v, w2_ops)

        def transpose_body(j, carry):
            pump(2, j, W // G)
            cols = pl.ds(pl.multiple_of(j * G, G), G)
            pt_s[cols, :] = p_s[:, cols].T.astype(_BF16)
            dst_s[cols, :] = ds_s[:, cols].T.astype(_BF16)
            return carry
        jax.lax.fori_loop(0, W // G, transpose_body, 0)

        grow = jax.lax.broadcasted_iota(jnp.int32, (G, 1), 0)

        def window_body(i, carry):
            pump(12, i, B * Hkv)
            b, h = i // Hkv, i % Hkv
            mine = jnp.logical_and((grow // R) % Hkv == h, (grow % R) // REP == b)
            qm = jnp.where(mine, q_s[...], 0.0).astype(_BF16)
            dom = jnp.where(mine, do_s[...], 0.0).astype(_BF16)
            for c in range(0, W, 512):
                dk_v[b, h, pl.ds(c, 512), :] = _mm(dst_s[pl.ds(c, 512), :], qm).astype(_BF16)
                dv_v[b, h, pl.ds(c, 512), :] = _mm(pt_s[pl.ds(c, 512), :], dom).astype(_BF16)
            return carry
        jax.lax.fori_loop(0, B * Hkv, window_body, 0)

        results = [
            pltpu.make_async_copy(out_v, out_hbm, wsem),
            pltpu.make_async_copy(dx_v, dx_hbm, wsem),
            pltpu.make_async_copy(db1_v, db1_hbm, wsem),
            pltpu.make_async_copy(db2_v, db2_hbm, wsem),
            pltpu.make_async_copy(dwq_v, dwq_hbm, wsem),
            pltpu.make_async_copy(dwo_v, dwo_hbm, wsem),
            pltpu.make_async_copy(dw1_v, dw1_hbm, wsem),
            pltpu.make_async_copy(dw2_v, dw2_hbm, wsem),
        ]
        for c in results:
            c.start()

        def window_writes(src_v, dst_hbm):
            def body(i, carry):
                grp, j = i // NWJ, i % NWJ
                b, h0 = grp // (Hkv // _ZHEADS), (grp % (Hkv // _ZHEADS)) * _ZHEADS
                r0 = pl.multiple_of(j * _ZROWS, _ZROWS)
                cache_write(src_v.at[b, pl.ds(h0, _ZHEADS), pl.ds(r0, _ZROWS), :],
                            dst_hbm, grp, pl.multiple_of(Sk - W + r0, _ZROWS)).start()
                return carry
            jax.lax.fori_loop(0, NG * NWJ, body, 0)

        def zero_writes(dst_hbm, z0):
            def body(z, carry):
                zero_write(dst_hbm, z).start()
                return carry
            jax.lax.fori_loop(z0, NZ, body, 0)

        window_writes(dk_v, dk_hbm)
        window_writes(dv_v, dv_hbm)
        zero_writes(dk_hbm, issued[0])
        zero_writes(dv_hbm, 0)

        for c in results:
            c.wait()
        pltpu.make_async_copy(dk_hbm, dk_hbm, wsem).wait()
        pltpu.make_async_copy(dv_hbm, dv_hbm, wsem).wait()

    def like(a):
        return jax.ShapeDtypeStruct(a.shape, a.dtype)

    def vmem_like(a):
        return pltpu.VMEM(a.shape, a.dtype)

    hbm = pl.BlockSpec(memory_space=pltpu.HBM)
    window = pltpu.VMEM((B, Hkv, W, Dh), _BF16)
    return tuple(pl.pallas_call(
        kernel,
        out_shape=[like(a) for a in (A_x, A_x, A_k_cache, A_v_cache, A_wq, A_wo,
                                     B_w1, B_b1, B_w2, B_b2)],
        in_specs=[hbm] * 10,
        out_specs=[hbm] * 10,
        scratch_shapes=[
            window, window, vmem_like(A_wq), vmem_like(A_wo), vmem_like(B_w1), vmem_like(B_w2),
            vmem_like(A_x), vmem_like(grad_out), vmem_like(B_b1), vmem_like(B_b2),
            window, window, vmem_like(A_wq), vmem_like(A_wo), vmem_like(B_w1), vmem_like(B_w2),
            vmem_like(A_x), vmem_like(A_x), vmem_like(B_b1), vmem_like(B_b2),
            pltpu.VMEM((_ZHEADS, _ZROWS, Dh), _BF16),
            pltpu.VMEM((G, W), _F32), pltpu.VMEM((G, W), _F32),
            pltpu.VMEM((W, G), _BF16), pltpu.VMEM((W, G), _BF16),
            pltpu.VMEM((G, Dh), _F32), pltpu.VMEM((G, Dh), _F32),
            pltpu.VMEM((G, Dh), _F32), pltpu.VMEM((G, Dh), _F32),
            pltpu.SemaphoreType.DMA((10,)), pltpu.SemaphoreType.DMA(()),
        ],
        compiler_params=pltpu.CompilerParams(vmem_limit_bytes=120 * 1024 * 1024),
    )(A_x, A_k_cache, A_v_cache, A_wq, A_wo, B_w1, B_b1, B_w2, B_b2, grad_out))
```

```python
import math

import jax
import jax.numpy as jnp
import jax.experimental.pallas as pl
import jax.experimental.pallas.tpu as pltpu

_F32 = jnp.float32
_BF16 = jnp.bfloat16

_ZHEADS = 8
_ZROWS = 112
_WROWS = 64


def _mm(a, b):
    return jax.lax.dot_general(a, b, (((1,), (0,)), ((), ())), preferred_element_type=_F32)


def _mm_nt(a, b):
    return jax.lax.dot_general(a, b, (((1,), (1,)), ((), ())), preferred_element_type=_F32)


def _ln_fwd(x, eps=1e-5):
    xc = x - jnp.mean(x, axis=-1, keepdims=True)
    var = jnp.mean(xc * xc, axis=-1, keepdims=True)
    rstd = 1.0 / jnp.sqrt(var + eps)
    return xc * rstd, rstd


def _ln_bwd(dy, y, rstd):
    return rstd * (dy - jnp.mean(dy, axis=-1, keepdims=True)
                   - y * jnp.mean(dy * y, axis=-1, keepdims=True))


_GELU_C = math.sqrt(2.0 / math.pi)
_GELU_A = 0.044715


def _gelu_and_grad(h):
    t = jnp.tanh(_GELU_C * (h + _GELU_A * h * h * h))
    cdf = 0.5 * (1.0 + t)
    dcdf = 0.5 * (1.0 - t * t) * _GELU_C * (1.0 + 3.0 * _GELU_A * h * h)
    return h * cdf, cdf + h * dcdf


@jax.jit
def pallas_interleave_layers__sliding_block_cached__dense_activation_gelu__decode_kernel(
    A_x: jax.Array,
    A_k_cache: jax.Array,
    A_v_cache: jax.Array,
    A_wq: jax.Array,
    A_wo: jax.Array,
    B_x: jax.Array,
    B_w1: jax.Array,
    B_b1: jax.Array,
    B_w2: jax.Array,
    B_b2: jax.Array,
    grad_out: jax.Array,
):
    del B_x
    B, Sq, D = A_x.shape
    _, Hkv, Sk, Dh = A_k_cache.shape
    HD = A_wq.shape[1]
    Hq = HD // Dh
    F = B_w1.shape[1]
    W = min(4096, max(256, Sk // 4))
    REP = Hq // Hkv
    R = B * REP
    NL = 2
    G = NL * Hkv * R
    assert (B, Sq, REP, R, Dh, G) == (2, 1, 4, 8, 128, 128)
    assert Hkv % _ZHEADS == 0 and (Sk - W) % _ZROWS == 0 and W % _WROWS == 0
    scale = Dh ** -0.5
    NG = B * Hkv // _ZHEADS
    NZJ = (Sk - W) // _ZROWS
    NWJ = W // _WROWS
    NZ = NG * NZJ

    def kernel(x_hbm, k_hbm, v_hbm, wq_hbm, wo_hbm, w1_hbm, b1_hbm, w2_hbm, b2_hbm, g_hbm,
               out_hbm, dx_hbm, dk_hbm, dv_hbm, dwq_hbm, dwo_hbm, dw1_hbm, db1_hbm, dw2_hbm, db2_hbm,
               k_v, v_v, wq_v, wo_v, w1_v, w2_v, x_v, g_v, b1_v, b2_v,
               dk_v, dv_v, dwq_v, dwo_v, dw1_v, dw2_v, out_v, dx_v, db1_v, db2_v,
               zero_v, p_s, ds_s, pt_s, dst_s, q_s, o_s, do_s, dq_s,
               rsem, wsem):
        reads = [
            pltpu.make_async_copy(k_hbm.at[:, :, pl.ds(Sk - W, W), :], k_v, rsem.at[0]),
            pltpu.make_async_copy(v_hbm.at[:, :, pl.ds(Sk - W, W), :], v_v, rsem.at[1]),
            pltpu.make_async_copy(x_hbm, x_v, rsem.at[2]),
            pltpu.make_async_copy(g_hbm, g_v, rsem.at[3]),
            pltpu.make_async_copy(b1_hbm, b1_v, rsem.at[4]),
            pltpu.make_async_copy(b2_hbm, b2_v, rsem.at[5]),
            pltpu.make_async_copy(wq_hbm, wq_v, rsem.at[6]),
            pltpu.make_async_copy(wo_hbm, wo_v, rsem.at[7]),
            pltpu.make_async_copy(w1_hbm, w1_v, rsem.at[8]),
            pltpu.make_async_copy(w2_hbm, w2_v, rsem.at[9]),
        ]
        for c in reads:
            c.start()
        zero_v[...] = jnp.zeros(zero_v.shape, zero_v.dtype)
        for c in reads:
            c.wait()

        def cache_write(src, dst_hbm, grp, row0, nrows):
            b, h0 = grp // (Hkv // _ZHEADS), (grp % (Hkv // _ZHEADS)) * _ZHEADS
            return pltpu.make_async_copy(
                src, dst_hbm.at[b, pl.ds(h0, _ZHEADS), pl.ds(row0, nrows), :], wsem)

        def zero_write(dst_hbm, z):
            return cache_write(zero_v, dst_hbm, z // NZJ,
                               pl.multiple_of((z % NZJ) * _ZROWS, 16), _ZROWS)

        issued = [0]

        def pump(n, i=0, trips=1):
            base = issued[0]
            assert base + n * trips <= NZ
            for j in range(n):
                zero_write(dk_hbm, base + i * n + j).start()
            issued[0] = base + n * trips

        row = jax.lax.broadcasted_iota(jnp.int32, (R, 1), 0)
        first_b = row < REP
        row_r = row % REP

        def per_batch(a0, a1):
            return jnp.where(first_b, a0, a1)

        def load_rep(ref):
            a = ref[...].astype(_F32)
            return per_batch(a[0:1], a[1:2])

        def store_rep(ref, a):
            ref[...] = jnp.concatenate([a[0:1], a[REP:REP + 1]], axis=0).astype(_BF16)

        def sum_r(a):
            s0 = jnp.sum(jnp.where(first_b, a, 0.0), axis=0, keepdims=True)
            s1 = jnp.sum(jnp.where(first_b, 0.0, a), axis=0, keepdims=True)
            return per_batch(s0, s1)

        def store_heads(dst, l, a_rep):
            for h in range(Hkv):
                t = a_rep[:, (h * REP) * Dh:(h * REP + 1) * Dh]
                for r in range(1, REP):
                    t = jnp.where(row_r == r, a_rep[:, (h * REP + r) * Dh:(h * REP + r + 1) * Dh], t)
                dst[pl.ds((l * Hkv + h) * R, R), :] = t

        def load_masked(src, l):
            parts = []
            for h in range(Hkv):
                t = src[pl.ds((l * Hkv + h) * R, R), :]
                parts += [jnp.where(row_r == r, t, 0.0) for r in range(REP)]
            return jnp.concatenate(parts, axis=1).astype(_BF16)

        def attn_fwd(l):
            def body(h, carry):
                pump(ATT_PUMP, h, Hkv)
                rows = pl.ds(pl.multiple_of((l * Hkv + h) * R, R), R)
                q = q_s[rows, :].astype(_BF16)
                s = per_batch(_mm_nt(q, k_v[0, h]), _mm_nt(q, k_v[1, h])) * scale
                e = jnp.exp(s - jnp.max(s, axis=-1, keepdims=True))
                p = e / jnp.sum(e, axis=-1, keepdims=True)
                p_s[rows, :] = p
                pb = p.astype(_BF16)
                o_s[rows, :] = per_batch(_mm(pb, v_v[0, h]), _mm(pb, v_v[1, h]))
                return carry
            jax.lax.fori_loop(0, Hkv, body, 0)

        def attn_bwd(l):
            def body(h, carry):
                pump(ATT_PUMP, h, Hkv)
                rows = pl.ds(pl.multiple_of((l * Hkv + h) * R, R), R)
                do = do_s[rows, :].astype(_BF16)
                dp = per_batch(_mm_nt(do, v_v[0, h]), _mm_nt(do, v_v[1, h]))
                p = p_s[rows, :]
                ds = p * (dp - jnp.sum(p * dp, axis=-1, keepdims=True)) * scale
                ds_s[rows, :] = ds
                dsb = ds.astype(_BF16)
                dq_s[rows, :] = per_batch(_mm(dsb, k_v[0, h]), _mm(dsb, k_v[1, h]))
                return carry
            jax.lax.fori_loop(0, Hkv, body, 0)

        ATT_PUMP = 6
        pump(32)
        b1 = b1_v[...].astype(_F32).reshape(1, F)
        b2 = b2_v[...].astype(_F32).reshape(1, D)

        x = load_rep(x_v)
        saved = []
        for l in range(NL):
            ya, rstd_a = _ln_fwd(x)
            ya_b = ya.astype(_BF16)
            store_heads(q_s, l, _mm(ya_b, wq_v[...]))
            pump(4)
            attn_fwd(l)
            o_b = load_masked(o_s, l)
            x = x + sum_r(_mm(o_b, wo_v[...]))
            pump(4)
            yb, rstd_b = _ln_fwd(x)
            yb_b = yb.astype(_BF16)
            act, dact = _gelu_and_grad(_mm(yb_b, w1_v[...]) + b1)
            act_b = act.astype(_BF16)
            x = x + _mm(act_b, w2_v[...]) + b2
            pump(4)
            saved.append((ya, rstd_a, ya_b, o_b, yb, rstd_b, yb_b, act_b, dact))
        store_rep(out_v, x)

        once = row_r == 0
        dx = load_rep(g_v)
        db1 = jnp.zeros((1, F), _F32)
        db2 = jnp.zeros((1, D), _F32)
        wq_ops, wo_ops, w1_ops, w2_ops = [], [], [], []
        for l in reversed(range(NL)):
            ya, rstd_a, ya_b, o_b, yb, rstd_b, yb_b, act_b, dact = saved[l]
            dx_once = jnp.where(once, dx, 0.0)
            db2 = db2 + jnp.sum(dx_once, axis=0, keepdims=True)
            w2_ops.append((act_b, dx_once.astype(_BF16)))
            dh = _mm_nt(dx.astype(_BF16), w2_v[...]) * dact
            dh_once = jnp.where(once, dh, 0.0)
            db1 = db1 + jnp.sum(dh_once, axis=0, keepdims=True)
            w1_ops.append((yb_b, dh_once.astype(_BF16)))
            dx = dx + _ln_bwd(_mm_nt(dh.astype(_BF16), w1_v[...]), yb, rstd_b)
            pump(4)
            dx_b = dx.astype(_BF16)
            wo_ops.append((o_b, dx_b))
            store_heads(do_s, l, _mm_nt(dx_b, wo_v[...]))
            pump(4)
            attn_bwd(l)
            dq_b = load_masked(dq_s, l)
            wq_ops.append((ya_b, dq_b))
            dx = dx + _ln_bwd(sum_r(_mm_nt(dq_b, wq_v[...])), ya, rstd_a)
            pump(4)
        store_rep(dx_v, dx)
        db1_v[...] = db1.reshape(F).astype(_BF16)
        db2_v[...] = db2.reshape(D).astype(_BF16)

        def weight_grad(dst, ops):
            a = jnp.concatenate([o[0].astype(_F32) for o in ops], axis=0)
            b = jnp.concatenate([o[1] for o in ops], axis=0)
            n, m = dst.shape
            for i in range(0, n, 512):
                sz = min(512, n - i)
                at = a[:, i:i + sz].T.astype(_BF16)
                for j in range(0, m, 1024):
                    sm = min(1024, m - j)
                    dst[i:i + sz, j:j + sm] = _mm(at, b[:, j:j + sm]).astype(_BF16)
                    pump(2)

        weight_grad(dwq_v, wq_ops)
        weight_grad(dwo_v, wo_ops)
        weight_grad(dw1_v, w1_ops)
        weight_grad(dw2_v, w2_ops)

        def transpose_body(j, carry):
            pump(1, j, W // G)
            cols = pl.ds(pl.multiple_of(j * G, G), G)
            pt_s[cols, :] = p_s[:, cols].T.astype(_BF16)
            dst_s[cols, :] = ds_s[:, cols].T.astype(_BF16)
            return carry
        jax.lax.fori_loop(0, W // G, transpose_body, 0)

        grow = jax.lax.broadcasted_iota(jnp.int32, (G, 1), 0)

        def window_body(i, carry):
            pump(6, i, B * Hkv)
            b, h = i // Hkv, i % Hkv
            mine = jnp.logical_and((grow // R) % Hkv == h, (grow % R) // REP == b)
            qm = jnp.where(mine, q_s[...], 0.0).astype(_BF16)
            dom = jnp.where(mine, do_s[...], 0.0).astype(_BF16)
            for c in range(0, W, 512):
                dk_v[b, h, pl.ds(c, 512), :] = _mm(dst_s[pl.ds(c, 512), :], qm).astype(_BF16)
                dv_v[b, h, pl.ds(c, 512), :] = _mm(pt_s[pl.ds(c, 512), :], dom).astype(_BF16)
            return carry
        jax.lax.fori_loop(0, B * Hkv, window_body, 0)

        results = [
            pltpu.make_async_copy(out_v, out_hbm, wsem),
            pltpu.make_async_copy(dx_v, dx_hbm, wsem),
            pltpu.make_async_copy(db1_v, db1_hbm, wsem),
            pltpu.make_async_copy(db2_v, db2_hbm, wsem),
        ]
        for c in results:
            c.start()

        def weight_writes(src, dst, streams=4):
            n, m = src.shape
            s3, d3 = src.reshape(streams, n // streams, m), dst.reshape(streams, n // streams, m)
            cols = m if m <= 1024 else (1024 if m % 1024 == 0 else m // 2)
            rows = max(16, (16384 // cols) // 16 * 16)
            def body(i, carry):
                r0 = pl.multiple_of(i * rows, rows)
                for c in range(0, m, cols):
                    pltpu.make_async_copy(s3.at[:, pl.ds(r0, rows), pl.ds(c, cols)],
                                          d3.at[:, pl.ds(r0, rows), pl.ds(c, cols)], wsem).start()
                return carry
            jax.lax.fori_loop(0, n // streams // rows, body, 0)

        weight_writes(dwq_v, dwq_hbm)
        weight_writes(dwo_v, dwo_hbm)
        weight_writes(dw1_v, dw1_hbm)
        weight_writes(dw2_v, dw2_hbm)

        def window_writes(src_v, dst_hbm):
            def body(i, carry):
                grp, j = i // NWJ, i % NWJ
                b, h0 = grp // (Hkv // _ZHEADS), (grp % (Hkv // _ZHEADS)) * _ZHEADS
                r0 = pl.multiple_of(j * _WROWS, _WROWS)
                cache_write(src_v.at[b, pl.ds(h0, _ZHEADS), pl.ds(r0, _WROWS), :],
                            dst_hbm, grp, pl.multiple_of(Sk - W + r0, _WROWS), _WROWS).start()
                return carry
            jax.lax.fori_loop(0, NG * NWJ, body, 0)

        def zero_writes(dst_hbm, z0):
            def body(z, carry):
                zero_write(dst_hbm, z).start()
                return carry
            jax.lax.fori_loop(z0, NZ, body, 0)

        window_writes(dk_v, dk_hbm)
        window_writes(dv_v, dv_hbm)
        zero_writes(dk_hbm, issued[0])
        zero_writes(dv_hbm, 0)

        for c in results:
            c.wait()
        for d in (dwq_hbm, dwo_hbm, dw1_hbm, dw2_hbm, dk_hbm, dv_hbm):
            pltpu.make_async_copy(d, d, wsem).wait()

    def like(a):
        return jax.ShapeDtypeStruct(a.shape, a.dtype)

    def vmem_like(a):
        return pltpu.VMEM(a.shape, a.dtype)

    hbm = pl.BlockSpec(memory_space=pltpu.HBM)
    window = pltpu.VMEM((B, Hkv, W, Dh), _BF16)
    x2, g2 = A_x.reshape(B, D), grad_out.reshape(B, D)
    out, dx, *grads = pl.pallas_call(
        kernel,
        out_shape=[like(a) for a in (x2, x2, A_k_cache, A_v_cache, A_wq, A_wo,
                                     B_w1, B_b1, B_w2, B_b2)],
        in_specs=[hbm] * 10,
        out_specs=[hbm] * 10,
        scratch_shapes=[
            window, window, vmem_like(A_wq), vmem_like(A_wo), vmem_like(B_w1), vmem_like(B_w2),
            vmem_like(x2), vmem_like(g2), vmem_like(B_b1), vmem_like(B_b2),
            window, window, vmem_like(A_wq), vmem_like(A_wo), vmem_like(B_w1), vmem_like(B_w2),
            vmem_like(x2), vmem_like(x2), vmem_like(B_b1), vmem_like(B_b2),
            pltpu.VMEM((_ZHEADS, _ZROWS, Dh), _BF16),
            pltpu.VMEM((G, W), _F32), pltpu.VMEM((G, W), _F32),
            pltpu.VMEM((W, G), _BF16), pltpu.VMEM((W, G), _BF16),
            pltpu.VMEM((G, Dh), _F32), pltpu.VMEM((G, Dh), _F32),
            pltpu.VMEM((G, Dh), _F32), pltpu.VMEM((G, Dh), _F32),
            pltpu.SemaphoreType.DMA((10,)), pltpu.SemaphoreType.DMA(()),
        ],
        compiler_params=pltpu.CompilerParams(vmem_limit_bytes=120 * 1024 * 1024),
    )(x2, A_k_cache, A_v_cache, A_wq, A_wo, B_w1, B_b1, B_w2, B_b2, g2)
    return (out.reshape(A_x.shape), dx.reshape(A_x.shape), *grads)
```

```python
import math

import jax
import jax.numpy as jnp
import jax.experimental.pallas as pl
import jax.experimental.pallas.tpu as pltpu

_F32 = jnp.float32
_BF16 = jnp.bfloat16

_ZERO_ROWS = 112
_WINDOW_ROWS = 64
_TAIL_ROWS = 96
_ATTN_STREAMS = 8
_MLP_STREAMS = 2

_GELU_C = math.sqrt(2.0 / math.pi)
_GELU_A = 0.044715


def _mm(a, b):
    return jax.lax.dot_general(a, b, (((1,), (0,)), ((), ())), preferred_element_type=_F32)


def _mm_nt(a, b):
    return jax.lax.dot_general(a, b, (((1,), (1,)), ((), ())), preferred_element_type=_F32)


def _ln_fwd(x, eps=1e-5):
    xc = x - jnp.mean(x, axis=-1, keepdims=True)
    var = jnp.mean(xc * xc, axis=-1, keepdims=True)
    rstd = 1.0 / jnp.sqrt(var + eps)
    return xc * rstd, rstd


def _ln_bwd(dy, y, rstd):
    return rstd * (dy - jnp.mean(dy, axis=-1, keepdims=True)
                   - y * jnp.mean(dy * y, axis=-1, keepdims=True))


def _gelu_and_grad(h):
    t = jnp.tanh(_GELU_C * (h + _GELU_A * h * h * h))
    cdf = 0.5 * (1.0 + t)
    dcdf = 0.5 * (1.0 - t * t) * _GELU_C * (1.0 + 3.0 * _GELU_A * h * h)
    return h * cdf, cdf + h * dcdf


def _loop(n, body):
    jax.lax.fori_loop(0, n, lambda i, carry: body(i), None)


@jax.jit
def pallas_interleave_layers__sliding_block_cached__dense_activation_gelu__decode_kernel(
    A_x: jax.Array,
    A_k_cache: jax.Array,
    A_v_cache: jax.Array,
    A_wq: jax.Array,
    A_wo: jax.Array,
    B_x: jax.Array,
    B_w1: jax.Array,
    B_b1: jax.Array,
    B_w2: jax.Array,
    B_b2: jax.Array,
    grad_out: jax.Array,
):
    del B_x
    B, Sq, D = A_x.shape
    _, Hkv, Sk, Dh = A_k_cache.shape
    HD = A_wq.shape[1]
    F = B_w1.shape[1]
    W = min(4096, max(256, Sk // 4))
    REP = HD // Dh // Hkv
    R = B * REP
    NL = 2
    G = NL * Hkv * R
    assert (B, Sq, REP, Dh, G) == (2, 1, 4, 128, 128)
    assert (Sk - W) % _ZERO_ROWS == 0 and W % _WINDOW_ROWS == 0
    scale = Dh ** -0.5
    NZJ = (Sk - W) // _ZERO_ROWS
    NZ = B * NZJ
    NWJ = W // _WINDOW_ROWS

    def kernel(x_hbm, k_hbm, v_hbm, wq_hbm, wo_hbm, w1_hbm, b1_hbm, w2_hbm, b2_hbm, g_hbm,
               out_hbm, dx_hbm, dk_hbm, dv_hbm, dwq_hbm, dwo_hbm, dw1_hbm, db1_hbm, dw2_hbm, db2_hbm,
               x_v, k_v, v_v, wq_v, wo_v, w1_v, b1_v, w2_v, b2_v, g_v,
               out_v, dx_v, dk_v, dv_v, dwq_v, dwo_v, dw1_v, db1_v, dw2_v, db2_v,
               zero_v, p_s, ds_s, pt_s, dst_s, q_s, o_s, do_s, dq_s,
               rsem, wsem):
        head_rows = W - _TAIL_ROWS
        reads = [
            (k_hbm.at[:, :, pl.ds(Sk - W, W), :], k_v),
            (x_hbm, x_v), (g_hbm, g_v), (b1_hbm, b1_v), (b2_hbm, b2_v),
            (wq_hbm, wq_v), (wo_hbm, wo_v), (w1_hbm, w1_v), (w2_hbm, w2_v),
            (v_hbm.at[:, :, pl.ds(Sk - W, head_rows), :], v_v.at[:, :, pl.ds(0, head_rows), :]),
            (v_hbm.at[:, :, pl.ds(Sk - _TAIL_ROWS, _TAIL_ROWS), :],
             v_v.at[:, :, pl.ds(head_rows, _TAIL_ROWS), :]),
        ]
        reads = [pltpu.make_async_copy(src, dst, rsem.at[i]) for i, (src, dst) in enumerate(reads)]
        for c in reads:
            c.start()
        zero_v[...] = jnp.zeros(zero_v.shape, zero_v.dtype)
        for c in reads[:-1]:
            c.wait()

        def write(src, dst):
            pltpu.make_async_copy(src, dst, wsem).start()

        def write_zeros(dst_hbm, z):
            rows = pl.ds(pl.multiple_of((z % NZJ) * _ZERO_ROWS, 16), _ZERO_ROWS)
            write(zero_v, dst_hbm.at[z // NZJ, :, rows, :])

        issued = [0]

        def pump(n, i=0, trips=1):
            for j in range(n):
                write_zeros(dk_hbm, issued[0] + i * n + j)
            issued[0] += n * trips
            assert issued[0] <= NZ

        pump(32)
        reads[-1].wait()

        row = jax.lax.broadcasted_iota(jnp.int32, (R, 1), 0)
        first_b = row < REP
        row_r = row % REP

        def per_batch(a0, a1):
            return jnp.where(first_b, a0, a1)

        def load_rep(ref):
            a = ref[...].astype(_F32)
            return per_batch(a[0:1], a[1:2])

        def store_rep(ref, a):
            ref[...] = jnp.concatenate([a[0:1], a[REP:REP + 1]], axis=0).astype(_BF16)

        def sum_r(a):
            s0 = jnp.sum(jnp.where(first_b, a, 0.0), axis=0, keepdims=True)
            s1 = jnp.sum(jnp.where(first_b, 0.0, a), axis=0, keepdims=True)
            return per_batch(s0, s1)

        def store_heads(dst, l, a):
            for h in range(Hkv):
                t = a[:, h * REP * Dh:(h * REP + 1) * Dh]
                for r in range(1, REP):
                    t = jnp.where(row_r == r, a[:, (h * REP + r) * Dh:(h * REP + r + 1) * Dh], t)
                dst[pl.ds((l * Hkv + h) * R, R), :] = t

        def load_masked(src, l):
            parts = []
            for h in range(Hkv):
                t = src[pl.ds((l * Hkv + h) * R, R), :]
                parts += [jnp.where(row_r == r, t, 0.0) for r in range(REP)]
            return jnp.concatenate(parts, axis=1).astype(_BF16)

        def attn_fwd(l):
            def body(h):
                pump(6, h, Hkv)
                rows = pl.ds(pl.multiple_of((l * Hkv + h) * R, R), R)
                q = q_s[rows, :].astype(_BF16)
                s = per_batch(_mm_nt(q, k_v[0, h]), _mm_nt(q, k_v[1, h])) * scale
                e = jnp.exp(s - jnp.max(s, axis=-1, keepdims=True))
                p = e / jnp.sum(e, axis=-1, keepdims=True)
                p_s[rows, :] = p
                p = p.astype(_BF16)
                o_s[rows, :] = per_batch(_mm(p, v_v[0, h]), _mm(p, v_v[1, h]))
            _loop(Hkv, body)

        def attn_bwd(l):
            def body(h):
                pump(6, h, Hkv)
                rows = pl.ds(pl.multiple_of((l * Hkv + h) * R, R), R)
                do = do_s[rows, :].astype(_BF16)
                dp = per_batch(_mm_nt(do, v_v[0, h]), _mm_nt(do, v_v[1, h]))
                p = p_s[rows, :]
                ds = p * (dp - jnp.sum(p * dp, axis=-1, keepdims=True)) * scale
                ds_s[rows, :] = ds
                ds = ds.astype(_BF16)
                dq_s[rows, :] = per_batch(_mm(ds, k_v[0, h]), _mm(ds, k_v[1, h]))
            _loop(Hkv, body)

        b1 = b1_v[...].astype(_F32).reshape(1, F)
        b2 = b2_v[...].astype(_F32).reshape(1, D)
        x = load_rep(x_v)
        saved = []
        for l in range(NL):
            ya, rstd_a = _ln_fwd(x)
            store_heads(q_s, l, _mm(ya.astype(_BF16), wq_v[...]))
            pump(4)
            attn_fwd(l)
            o = load_masked(o_s, l)
            x = x + sum_r(_mm(o, wo_v[...]))
            pump(4)
            yb, rstd_b = _ln_fwd(x)
            act, dact = _gelu_and_grad(_mm(yb.astype(_BF16), w1_v[...]) + b1)
            x = x + _mm(act.astype(_BF16), w2_v[...]) + b2
            pump(4)
            saved.append((ya, rstd_a, o, yb, rstd_b, act, dact))
        store_rep(out_v, x)

        def once(a):
            return jnp.where(row_r == 0, a, 0.0)

        dx = load_rep(g_v)
        db1 = jnp.zeros((1, F), _F32)
        db2 = jnp.zeros((1, D), _F32)
        wq_ops, wo_ops, w1_ops, w2_ops = [], [], [], []
        for l in reversed(range(NL)):
            ya, rstd_a, o, yb, rstd_b, act, dact = saved[l]
            db2 = db2 + jnp.sum(once(dx), axis=0, keepdims=True)
            w2_ops.append((act, once(dx)))
            dh = _mm_nt(dx.astype(_BF16), w2_v[...]) * dact
            db1 = db1 + jnp.sum(once(dh), axis=0, keepdims=True)
            w1_ops.append((yb, once(dh)))
            dx = dx + _ln_bwd(_mm_nt(dh.astype(_BF16), w1_v[...]), yb, rstd_b)
            pump(4)
            wo_ops.append((o, dx))
            store_heads(do_s, l, _mm_nt(dx.astype(_BF16), wo_v[...]))
            pump(4)
            attn_bwd(l)
            dq = load_masked(dq_s, l)
            wq_ops.append((ya, dq))
            dx = dx + _ln_bwd(sum_r(_mm_nt(dq, wq_v[...])), ya, rstd_a)
            pump(4)
        store_rep(dx_v, dx)
        db1_v[...] = db1.reshape(F).astype(_BF16)
        db2_v[...] = db2.reshape(D).astype(_BF16)

        def weight_grad(dst, ops):
            a = jnp.concatenate([a.astype(_F32) for a, _ in ops], axis=0)
            b = jnp.concatenate([b.astype(_F32) for _, b in ops], axis=0).astype(_BF16)
            streams, rows, cols = dst.shape
            group = max(1, 512 // rows)
            for s in range(0, streams, group):
                at = a[:, s * rows:(s + group) * rows].T.astype(_BF16)
                for c in range(0, cols, 1024):
                    n = min(1024, cols - c)
                    g = _mm(at, b[:, c:c + n]).astype(_BF16)
                    dst[s:s + group, :, c:c + n] = g.reshape(group, rows, n)
                    pump(2)

        weight_grad(dwq_v, wq_ops)
        weight_grad(dwo_v, wo_ops)
        weight_grad(dw1_v, w1_ops)
        weight_grad(dw2_v, w2_ops)

        def transpose_body(j):
            pump(1, j, W // G)
            cols = pl.ds(pl.multiple_of(j * G, G), G)
            pt_s[cols, :] = p_s[:, cols].T.astype(_BF16)
            dst_s[cols, :] = ds_s[:, cols].T.astype(_BF16)
        _loop(W // G, transpose_body)

        def window_body(i):
            pump(6, i, B * Hkv)
            b, h = i // Hkv, i % Hkv
            g = jax.lax.broadcasted_iota(jnp.int32, (G, 1), 0)
            mine = jnp.logical_and((g // R) % Hkv == h, (g % R) // REP == b)
            q = jnp.where(mine, q_s[...], 0.0).astype(_BF16)
            do = jnp.where(mine, do_s[...], 0.0).astype(_BF16)
            for c in range(0, W, 512):
                dk_v[b, h, pl.ds(c, 512), :] = _mm(dst_s[pl.ds(c, 512), :], q).astype(_BF16)
                dv_v[b, h, pl.ds(c, 512), :] = _mm(pt_s[pl.ds(c, 512), :], do).astype(_BF16)
        _loop(B * Hkv, window_body)

        for src, dst in ((out_v, out_hbm), (dx_v, dx_hbm), (db1_v, db1_hbm), (db2_v, db2_hbm)):
            write(src, dst)

        def write_piece(src, dst, i, nrows, cols):
            rows = pl.ds(pl.multiple_of(i * nrows, nrows), nrows)
            write(src.at[:, rows, cols], dst.at[:, rows, cols])

        def wq_body(i):
            for c in range(0, HD, 1024):
                write_piece(dwq_v, dwq_hbm, i, 8, pl.ds(c, 1024))
        _loop(dwq_v.shape[1] // 8, wq_body)
        _loop(dwo_v.shape[1] // 16, lambda i: write_piece(dwo_v, dwo_hbm, i, 16, pl.ds(0, D)))

        n1, n2 = dw1_v.shape[1] // 8, dw2_v.shape[1] // 32
        assert n2 <= n1

        def mlp_body(i):
            write_piece(dw1_v, dw1_hbm, i, 8, pl.ds(0, F))
            pl.when(i < n2)(
                lambda: write_piece(dw2_v, dw2_hbm, jnp.minimum(i, n2 - 1), 32, pl.ds(0, D)))
        _loop(n1, mlp_body)

        def write_window(src, dst_hbm, i):
            b, r0 = i // NWJ, (i % NWJ) * _WINDOW_ROWS
            write(src.at[b, :, pl.ds(pl.multiple_of(r0, _WINDOW_ROWS), _WINDOW_ROWS), :],
                  dst_hbm.at[b, :, pl.ds(pl.multiple_of(Sk - W + r0, _WINDOW_ROWS), _WINDOW_ROWS), :])

        _loop(B * NWJ, lambda i: write_window(dk_v, dk_hbm, i))
        _loop(B * NWJ, lambda i: write_window(dv_v, dv_hbm, i))
        _loop(NZ - issued[0], lambda z: write_zeros(dk_hbm, issued[0] + z))
        _loop(NZ, lambda z: write_zeros(dv_hbm, z))

        for dst in (out_hbm, dx_hbm, dk_hbm, dv_hbm, dwq_hbm, dwo_hbm,
                    dw1_hbm, db1_hbm, dw2_hbm, db2_hbm):
            pltpu.make_async_copy(dst, dst, wsem).wait()

    def split_rows(a, streams):
        return (streams, a.shape[0] // streams, a.shape[1])

    window = (B, Hkv, W, Dh)
    grad_w = (split_rows(A_wq, _ATTN_STREAMS), split_rows(A_wo, _ATTN_STREAMS),
              split_rows(B_w1, _MLP_STREAMS), (F,), split_rows(B_w2, _MLP_STREAMS), (D,))
    staged = ((B, D), window, window, A_wq.shape, A_wo.shape,
              B_w1.shape, (F,), B_w2.shape, (D,), (B, D),
              (B, D), (B, D), window, window, *grad_w,
              (Hkv, _ZERO_ROWS, Dh))
    hbm = pl.BlockSpec(memory_space=pltpu.HBM)
    out, dx, dk, dv, dwq, dwo, dw1, db1, dw2, db2 = pl.pallas_call(
        kernel,
        out_shape=[jax.ShapeDtypeStruct(s, _BF16) for s in
                   ((B, D), (B, D), A_k_cache.shape, A_v_cache.shape, *grad_w)],
        in_specs=[hbm] * 10,
        out_specs=[hbm] * 10,
        scratch_shapes=[
            *(pltpu.VMEM(s, _BF16) for s in staged),
            pltpu.VMEM((G, W), _F32), pltpu.VMEM((G, W), _F32),
            pltpu.VMEM((W, G), _BF16), pltpu.VMEM((W, G), _BF16),
            *(pltpu.VMEM((G, Dh), _F32) for _ in range(4)),
            pltpu.SemaphoreType.DMA((11,)), pltpu.SemaphoreType.DMA(()),
        ],
        compiler_params=pltpu.CompilerParams(vmem_limit_bytes=120 * 1024 * 1024),
    )(A_x.reshape(B, D), A_k_cache, A_v_cache, A_wq, A_wo,
      B_w1, B_b1, B_w2, B_b2, grad_out.reshape(B, D))
    return (out.reshape(A_x.shape), dx.reshape(A_x.shape), dk, dv,
            dwq.reshape(A_wq.shape), dwo.reshape(A_wo.shape),
            dw1.reshape(B_w1.shape), db1, dw2.reshape(B_w2.shape), db2)
```

```python
import math

import jax
import jax.numpy as jnp
import jax.experimental.pallas as pl
import jax.experimental.pallas.tpu as pltpu

_F32 = jnp.float32
_BF16 = jnp.bfloat16

_ZERO_ROWS = 112
_WINDOW_ROWS = 64
_TAIL_ROWS = 96
_ATTN_STREAMS = 8
_MLP_STREAMS = 2

_GELU_C = math.sqrt(2.0 / math.pi)
_GELU_A = 0.044715


def _mm(a, b):
    return jax.lax.dot_general(a, b, (((1,), (0,)), ((), ())), preferred_element_type=_F32)


def _mm_nt(a, b):
    return jax.lax.dot_general(a, b, (((1,), (1,)), ((), ())), preferred_element_type=_F32)


def _ln_fwd(x, eps=1e-5):
    xc = x - jnp.mean(x, axis=-1, keepdims=True)
    var = jnp.mean(xc * xc, axis=-1, keepdims=True)
    rstd = 1.0 / jnp.sqrt(var + eps)
    return xc * rstd, rstd


def _ln_bwd(dy, y, rstd):
    return rstd * (dy - jnp.mean(dy, axis=-1, keepdims=True)
                   - y * jnp.mean(dy * y, axis=-1, keepdims=True))


def _gelu_and_grad(h):
    t = jnp.tanh(_GELU_C * (h + _GELU_A * h * h * h))
    cdf = 0.5 * (1.0 + t)
    dcdf = 0.5 * (1.0 - t * t) * _GELU_C * (1.0 + 3.0 * _GELU_A * h * h)
    return h * cdf, cdf + h * dcdf


def _loop(n, body):
    jax.lax.fori_loop(0, n, lambda i, carry: body(i), None)


@jax.jit
def pallas_interleave_layers__sliding_block_cached__dense_activation_gelu__decode_kernel(
    A_x: jax.Array,
    A_k_cache: jax.Array,
    A_v_cache: jax.Array,
    A_wq: jax.Array,
    A_wo: jax.Array,
    B_x: jax.Array,
    B_w1: jax.Array,
    B_b1: jax.Array,
    B_w2: jax.Array,
    B_b2: jax.Array,
    grad_out: jax.Array,
):
    del B_x
    B, Sq, D = A_x.shape
    _, Hkv, Sk, Dh = A_k_cache.shape
    HD = A_wq.shape[1]
    F = B_w1.shape[1]
    W = min(4096, max(256, Sk // 4))
    REP = HD // Dh // Hkv
    R = B * REP
    NL = 2
    G = NL * Hkv * R
    assert (B, Sq, REP, Dh, G) == (2, 1, 4, 128, 128)
    assert (Sk - W) % _ZERO_ROWS == 0 and W % _WINDOW_ROWS == 0
    scale = Dh ** -0.5
    NZJ = (Sk - W) // _ZERO_ROWS
    NZ = B * NZJ
    NWJ = W // _WINDOW_ROWS

    def kernel(x_hbm, k_hbm, v_hbm, wq_hbm, wo_hbm, w1_hbm, b1_hbm, w2_hbm, b2_hbm, g_hbm,
               out_hbm, dx_hbm, dk_hbm, dv_hbm, dwq_hbm, dwo_hbm, dw1_hbm, db1_hbm, dw2_hbm, db2_hbm,
               x_v, k_v, v_v, wq_v, wo_v, w1_v, b1_v, w2_v, b2_v, g_v,
               out_v, dx_v, dk_v, dv_v, dwq_v, dwo_v, dw1_v, db1_v, dw2_v, db2_v,
               zero_v, p_s, ds_s, pt_s, dst_s, q_s, o_s, do_s, dq_s,
               rsem, wsem):
        head_rows = W - _TAIL_ROWS
        reads = [
            (k_hbm.at[:, :, pl.ds(Sk - W, W), :], k_v),
            (x_hbm, x_v), (g_hbm, g_v), (b1_hbm, b1_v), (b2_hbm, b2_v),
            (wq_hbm, wq_v), (wo_hbm, wo_v), (w1_hbm, w1_v), (w2_hbm, w2_v),
            (v_hbm.at[:, :, pl.ds(Sk - W, head_rows), :], v_v.at[:, :, pl.ds(0, head_rows), :]),
            (v_hbm.at[:, :, pl.ds(Sk - _TAIL_ROWS, _TAIL_ROWS), :],
             v_v.at[:, :, pl.ds(head_rows, _TAIL_ROWS), :]),
        ]
        reads = [pltpu.make_async_copy(src, dst, rsem.at[i]) for i, (src, dst) in enumerate(reads)]
        for c in reads:
            c.start()
        zero_v[...] = jnp.zeros(zero_v.shape, zero_v.dtype)
        for c in reads[:-1]:
            c.wait()

        def write(src, dst):
            pltpu.make_async_copy(src, dst, wsem).start()

        def write_zeros(dst_hbm, z):
            rows = pl.ds(pl.multiple_of((z % NZJ) * _ZERO_ROWS, 16), _ZERO_ROWS)
            write(zero_v, dst_hbm.at[z // NZJ, :, rows, :])

        issued = [0]

        def pump(n):
            for z in range(issued[0], issued[0] + n):
                write_zeros(dk_hbm, z)
            issued[0] += n

        def pumped_loop(trips, n, body):
            base = issued[0]
            issued[0] += trips * n

            def step(i):
                for j in range(n):
                    write_zeros(dk_hbm, base + i * n + j)
                body(i)
            _loop(trips, step)

        pump(32)
        reads[-1].wait()

        row = jax.lax.broadcasted_iota(jnp.int32, (R, 1), 0)
        first_b = row < REP
        row_r = row % REP

        def per_batch(a0, a1):
            return jnp.where(first_b, a0, a1)

        def load_rep(ref):
            a = ref[...].astype(_F32)
            return per_batch(a[0:1], a[1:2])

        def store_rep(ref, a):
            ref[...] = jnp.concatenate([a[0:1], a[REP:REP + 1]], axis=0).astype(_BF16)

        def sum_r(a):
            s0 = jnp.sum(jnp.where(first_b, a, 0.0), axis=0, keepdims=True)
            s1 = jnp.sum(jnp.where(first_b, 0.0, a), axis=0, keepdims=True)
            return per_batch(s0, s1)

        def store_heads(dst, l, a):
            for h in range(Hkv):
                t = a[:, h * REP * Dh:(h * REP + 1) * Dh]
                for r in range(1, REP):
                    t = jnp.where(row_r == r, a[:, (h * REP + r) * Dh:(h * REP + r + 1) * Dh], t)
                dst[pl.ds((l * Hkv + h) * R, R), :] = t

        def load_masked(src, l):
            parts = []
            for h in range(Hkv):
                t = src[pl.ds((l * Hkv + h) * R, R), :]
                parts += [jnp.where(row_r == r, t, 0.0) for r in range(REP)]
            return jnp.concatenate(parts, axis=1).astype(_BF16)

        def attn_fwd(l):
            def body(h):
                rows = pl.ds(pl.multiple_of((l * Hkv + h) * R, R), R)
                q = q_s[rows, :].astype(_BF16)
                s = per_batch(_mm_nt(q, k_v[0, h]), _mm_nt(q, k_v[1, h])) * scale
                e = jnp.exp(s - jnp.max(s, axis=-1, keepdims=True))
                p = e / jnp.sum(e, axis=-1, keepdims=True)
                p_s[rows, :] = p
                p = p.astype(_BF16)
                o_s[rows, :] = per_batch(_mm(p, v_v[0, h]), _mm(p, v_v[1, h]))
            pumped_loop(Hkv, 6, body)

        def attn_bwd(l):
            def body(h):
                rows = pl.ds(pl.multiple_of((l * Hkv + h) * R, R), R)
                do = do_s[rows, :].astype(_BF16)
                dp = per_batch(_mm_nt(do, v_v[0, h]), _mm_nt(do, v_v[1, h]))
                p = p_s[rows, :]
                ds = p * (dp - jnp.sum(p * dp, axis=-1, keepdims=True)) * scale
                ds_s[rows, :] = ds
                ds = ds.astype(_BF16)
                dq_s[rows, :] = per_batch(_mm(ds, k_v[0, h]), _mm(ds, k_v[1, h]))
            pumped_loop(Hkv, 6, body)

        b1 = b1_v[...].astype(_F32).reshape(1, F)
        b2 = b2_v[...].astype(_F32).reshape(1, D)
        x = load_rep(x_v)
        saved = []
        for l in range(NL):
            ya, rstd_a = _ln_fwd(x)
            store_heads(q_s, l, _mm(ya.astype(_BF16), wq_v[...]))
            pump(4)
            attn_fwd(l)
            o = load_masked(o_s, l)
            x = x + sum_r(_mm(o, wo_v[...]))
            pump(4)
            yb, rstd_b = _ln_fwd(x)
            act, dact = _gelu_and_grad(_mm(yb.astype(_BF16), w1_v[...]) + b1)
            x = x + _mm(act.astype(_BF16), w2_v[...]) + b2
            pump(4)
            saved.append((ya, rstd_a, o, yb, rstd_b, act, dact))
        store_rep(out_v, x)

        def once(a):
            return jnp.where(row_r == 0, a, 0.0)

        dx = load_rep(g_v)
        db1 = jnp.zeros((1, F), _F32)
        db2 = jnp.zeros((1, D), _F32)
        wq_ops, wo_ops, w1_ops, w2_ops = [], [], [], []
        for l in reversed(range(NL)):
            ya, rstd_a, o, yb, rstd_b, act, dact = saved[l]
            db2 = db2 + jnp.sum(once(dx), axis=0, keepdims=True)
            w2_ops.append((act, once(dx)))
            dh = _mm_nt(dx.astype(_BF16), w2_v[...]) * dact
            db1 = db1 + jnp.sum(once(dh), axis=0, keepdims=True)
            w1_ops.append((yb, once(dh)))
            dx = dx + _ln_bwd(_mm_nt(dh.astype(_BF16), w1_v[...]), yb, rstd_b)
            pump(4)
            wo_ops.append((o, dx))
            store_heads(do_s, l, _mm_nt(dx.astype(_BF16), wo_v[...]))
            pump(4)
            attn_bwd(l)
            dq = load_masked(dq_s, l)
            wq_ops.append((ya, dq))
            dx = dx + _ln_bwd(sum_r(_mm_nt(dq, wq_v[...])), ya, rstd_a)
            pump(4)
        store_rep(dx_v, dx)
        db1_v[...] = db1.reshape(F).astype(_BF16)
        db2_v[...] = db2.reshape(D).astype(_BF16)

        def weight_grad(dst, ops):
            a = jnp.concatenate([a.astype(_F32) for a, _ in ops], axis=0)
            b = jnp.concatenate([b.astype(_F32) for _, b in ops], axis=0).astype(_BF16)
            streams, rows, cols = dst.shape
            group = max(1, 512 // rows)
            for s in range(0, streams, group):
                at = a[:, s * rows:(s + group) * rows].T.astype(_BF16)
                for c in range(0, cols, 1024):
                    n = min(1024, cols - c)
                    g = _mm(at, b[:, c:c + n]).astype(_BF16)
                    dst[s:s + group, :, c:c + n] = g.reshape(group, rows, n)
                    pump(2)

        weight_grad(dwq_v, wq_ops)
        weight_grad(dwo_v, wo_ops)
        weight_grad(dw1_v, w1_ops)
        weight_grad(dw2_v, w2_ops)

        def transpose_body(j):
            cols = pl.ds(pl.multiple_of(j * G, G), G)
            pt_s[cols, :] = p_s[:, cols].T.astype(_BF16)
            dst_s[cols, :] = ds_s[:, cols].T.astype(_BF16)
        pumped_loop(W // G, 1, transpose_body)

        def window_body(i):
            b, h = i // Hkv, i % Hkv
            g = jax.lax.broadcasted_iota(jnp.int32, (G, 1), 0)
            mine = jnp.logical_and((g // R) % Hkv == h, (g % R) // REP == b)
            q = jnp.where(mine, q_s[...], 0.0).astype(_BF16)
            do = jnp.where(mine, do_s[...], 0.0).astype(_BF16)
            for c in range(0, W, 512):
                dk_v[b, h, pl.ds(c, 512), :] = _mm(dst_s[pl.ds(c, 512), :], q).astype(_BF16)
                dv_v[b, h, pl.ds(c, 512), :] = _mm(pt_s[pl.ds(c, 512), :], do).astype(_BF16)
        pumped_loop(B * Hkv, 6, window_body)

        for src, dst in ((out_v, out_hbm), (dx_v, dx_hbm), (db1_v, db1_hbm), (db2_v, db2_hbm)):
            write(src, dst)

        def write_piece(src, dst, i, nrows, cols):
            rows = pl.ds(pl.multiple_of(i * nrows, nrows), nrows)
            write(src.at[:, rows, cols], dst.at[:, rows, cols])

        def wq_body(i):
            for c in range(0, HD, 1024):
                write_piece(dwq_v, dwq_hbm, i, 8, pl.ds(c, 1024))
        _loop(dwq_v.shape[1] // 8, wq_body)
        _loop(dwo_v.shape[1] // 16, lambda i: write_piece(dwo_v, dwo_hbm, i, 16, pl.ds(0, D)))

        n1, n2 = dw1_v.shape[1] // 8, dw2_v.shape[1] // 32
        assert n2 <= n1

        def mlp_body(i):
            write_piece(dw1_v, dw1_hbm, i, 8, pl.ds(0, F))
            pl.when(i < n2)(
                lambda: write_piece(dw2_v, dw2_hbm, jnp.minimum(i, n2 - 1), 32, pl.ds(0, D)))
        _loop(n1, mlp_body)

        def write_window(src, dst_hbm, i):
            b, r0 = i // NWJ, (i % NWJ) * _WINDOW_ROWS
            write(src.at[b, :, pl.ds(pl.multiple_of(r0, _WINDOW_ROWS), _WINDOW_ROWS), :],
                  dst_hbm.at[b, :, pl.ds(pl.multiple_of(Sk - W + r0, _WINDOW_ROWS), _WINDOW_ROWS), :])

        _loop(B * NWJ, lambda i: write_window(dk_v, dk_hbm, i))
        _loop(B * NWJ, lambda i: write_window(dv_v, dv_hbm, i))
        assert issued[0] < NZ
        pumped_loop(NZ - issued[0], 1, lambda i: None)
        _loop(NZ, lambda z: write_zeros(dv_hbm, z))

        for dst in (out_hbm, dx_hbm, dk_hbm, dv_hbm, dwq_hbm, dwo_hbm,
                    dw1_hbm, db1_hbm, dw2_hbm, db2_hbm):
            pltpu.make_async_copy(dst, dst, wsem).wait()

    def split_rows(a, streams):
        return (streams, a.shape[0] // streams, a.shape[1])

    window = (B, Hkv, W, Dh)
    grad_w = (split_rows(A_wq, _ATTN_STREAMS), split_rows(A_wo, _ATTN_STREAMS),
              split_rows(B_w1, _MLP_STREAMS), (F,), split_rows(B_w2, _MLP_STREAMS), (D,))
    staged = ((B, D), window, window, A_wq.shape, A_wo.shape,
              B_w1.shape, (F,), B_w2.shape, (D,), (B, D),
              (B, D), (B, D), window, window, *grad_w,
              (Hkv, _ZERO_ROWS, Dh))
    hbm = pl.BlockSpec(memory_space=pltpu.HBM)
    out, dx, dk, dv, dwq, dwo, dw1, db1, dw2, db2 = pl.pallas_call(
        kernel,
        out_shape=[jax.ShapeDtypeStruct(s, _BF16) for s in
                   ((B, D), (B, D), A_k_cache.shape, A_v_cache.shape, *grad_w)],
        in_specs=[hbm] * 10,
        out_specs=[hbm] * 10,
        scratch_shapes=[
            *(pltpu.VMEM(s, _BF16) for s in staged),
            pltpu.VMEM((G, W), _F32), pltpu.VMEM((G, W), _F32),
            pltpu.VMEM((W, G), _BF16), pltpu.VMEM((W, G), _BF16),
            *(pltpu.VMEM((G, Dh), _F32) for _ in range(4)),
            pltpu.SemaphoreType.DMA((11,)), pltpu.SemaphoreType.DMA(()),
        ],
        compiler_params=pltpu.CompilerParams(vmem_limit_bytes=120 * 1024 * 1024),
    )(A_x.reshape(B, D), A_k_cache, A_v_cache, A_wq, A_wo,
      B_w1, B_b1, B_w2, B_b2, grad_out.reshape(B, D))
    return (out.reshape(A_x.shape), dx.reshape(A_x.shape), dk, dv,
            dwq.reshape(A_wq.shape), dwo.reshape(A_wo.shape),
            dw1.reshape(B_w1.shape), db1, dw2.reshape(B_w2.shape), db2)
```
